```python
import os as _os
_os.environ.setdefault('JAX_PLATFORMS', 'cpu')
import jax
import jax.numpy as jnp

def _softmax(x, axis=-1):
    return jax.nn.softmax(x, axis=axis)

def _gelu(x):
    return jax.nn.gelu(x, approximate=True)

def _silu(x):
    return jax.nn.silu(x)

def _sigmoid(x):
    return jax.nn.sigmoid(x)

def _layernorm(x, axis=-1, eps=1e-05):
    m = jnp.mean(x, axis=axis, keepdims=True)
    v = jnp.var(x, axis=axis, keepdims=True)
    return (x - m) / jnp.sqrt(v + eps)

def _scatter_add(tgt, idx, src, axis=0):
    return tgt.at[idx].add(src)

def _segment_sum(src, seg, n):
    return jax.ops.segment_sum(src, seg, n)

class _Rng:

    def __init__(self, key):
        self._k = key

    def _next(self):
        self._k, sub = jax.random.split(self._k)
        return sub

    def normal(self, shape):
        return jax.random.normal(self._next(), shape, dtype=jnp.bfloat16)

    def randint(self, lo, hi, shape):
        return jax.random.randint(self._next(), shape, lo, hi, dtype=jnp.int32)

    def uniform(self, shape, lo=0.0, hi=1.0):
        return jax.random.uniform(self._next(), shape, jnp.bfloat16, lo, hi)

    def permutation(self, n):
        return jax.random.permutation(self._next(), n)
kernel_name = 'sequential_preLN__linear_attn_block__mixer_gmlp__prompt'

def setup_inputs():
    _rng = _Rng(jax.random.key(int.from_bytes(__import__("os").urandom(4), "little")))
    _w = lambda a: (lambda t: t.astype(jnp.bfloat16) if jnp.issubdtype(t.dtype, jnp.floating) else t)(jnp.asarray(a))

    def _A_setup():
        B, S, D = (1, 2048, 512)
        return {'x': _w((lambda *s: _rng.normal(s) * 0.05)(B, S, D)), 'wqkv': _w((lambda *s: _rng.normal(s) * 0.05)(D, 3 * D)), 'wo': _w((lambda *s: _rng.normal(s) * 0.05)(D, D))}
    _A_in = _A_setup()

    def _B_setup():
        B, S, D, F = (1, 2048, 512, 1792)
        Fh = F // 2
        return {'x': _w((lambda *s: _rng.normal(s) * 0.05)(B, S, D)), 'w_in': _w((lambda *s: _rng.normal(s) * 0.4)(D, 2 * Fh)), 'w_sp': _w(0.01 * (lambda *s: _rng.normal(s) * 0.4)(S, S)), 'b_sp': _w(1.0 + 0.01 * (lambda *s: _rng.normal(s) * 0.05)(S)), 'w_out': _w((lambda *s: _rng.normal(s) * 0.05)(Fh, D))}
    _B_in = _B_setup()
    return {'A_x': _A_in['x'], 'A_wqkv': _A_in['wqkv'], 'A_wo': _A_in['wo'], 'B_x': _B_in['x'], 'B_w_in': _B_in['w_in'], 'B_w_sp': _B_in['w_sp'], 'B_b_sp': _B_in['b_sp'], 'B_w_out': _B_in['w_out']}

def reference(A_x, A_wqkv, A_wo, B_x, B_w_in, B_w_sp, B_b_sp, B_w_out):

    def _A_ref(x, wqkv, wo):
        B, S, D = x.shape
        H = 32
        Dh = D // H
        qkv = (lambda x, *d: x.transpose(*d))((x @ wqkv).reshape(B, S, 3, H, Dh), 2, 0, 3, 1, 4)
        q, k, v = (qkv[0], qkv[1], qkv[2])
        phi = lambda t: jnp.where(t > 0, t + 1, jnp.exp(t)) + 1e-06
        pq, pk = (phi(q), phi(k))
        kv = jnp.einsum('bhsd,bhse->bhde', pk, v)
        z = jnp.einsum('bhsd->bhd', pk)
        num = jnp.einsum('bhqd,bhde->bhqe', pq, kv)
        den = jnp.einsum('bhqd,bhd->bhq', pq, z)[..., None] + 1e-06
        o = num / den
        return (lambda x, *d: x.transpose(*d))(o, 0, 2, 1, 3).reshape(B, S, D) @ wo

    def _B_ref(x, w_in, w_sp, b_sp, w_out):
        B, S, D = x.shape
        F = w_in.shape[-1]
        Fh = F // 2
        z = _gelu(jnp.einsum('bsd,df->bsf', x, w_in))
        z1 = z[..., :Fh].copy()
        z2 = _layernorm(z[..., Fh:], axis=-1)
        g = jnp.einsum('ts,bsf->btf', w_sp, z2) + b_sp[None, :, None]
        return jnp.einsum('bsf,fd->bsd', z1 * g, w_out)
    x = A_x
    h = x + _A_ref(_layernorm(x, axis=-1), A_wqkv, A_wo)
    h2 = h + _B_ref(_layernorm(h, axis=-1), B_w_in, B_w_sp, B_b_sp, B_w_out)
    return h2
```

```python
import functools
import jax
import jax.numpy as jnp
from jax import lax
import jax.experimental.pallas as pl
import jax.experimental.pallas.tpu as pltpu

S, D, H, DH = 2048, 512, 32, 16
F = 1792
FH = 896
TM = 256
NT = S // TM
f32 = jnp.float32
bf16 = jnp.bfloat16


def _ln(x):
    m = jnp.mean(x, axis=-1, keepdims=True)
    xc = x - m
    v = jnp.mean(xc * xc, axis=-1, keepdims=True)
    return xc * lax.rsqrt(v + 1e-5)


def _phi(t):
    return jnp.where(t > 0, t + 1.0, jnp.exp(t)) + 1e-6


def _gelu(x):
    c = 0.7978845608028654
    return 0.5 * x * (1.0 + jnp.tanh(c * (x + 0.044715 * (x * x * x))))


def _kernel(x_hbm, wqkv_hbm, wo_hbm, win_hbm, wsp_hbm, bsp_hbm, wout_hbm, o_hbm,
            x_v, wqkv_v, wo_v, win_v, wsp_v, bsp_v, wout_v,
            pq_v, h_v, z1_v, z2_v, kv_v, zs_v, m_v, bcol_v, o_v,
            xsem, wsem, osem):
    def x_copy(i):
        r = pl.multiple_of(i * TM, TM)
        return pltpu.make_async_copy(x_hbm.at[0, pl.ds(r, TM), :], x_v.at[pl.ds(r, TM), :], xsem.at[i])

    wq_cp = pltpu.make_async_copy(wqkv_hbm, wqkv_v, wsem.at[0])
    wo_cp = pltpu.make_async_copy(wo_hbm, wo_v, wsem.at[1])
    win_cp = pltpu.make_async_copy(win_hbm, win_v, wsem.at[2])
    wsp_cp = pltpu.make_async_copy(wsp_hbm, wsp_v, wsem.at[3])
    bsp_cp = pltpu.make_async_copy(bsp_hbm, bsp_v, wsem.at[4])
    wout_cp = pltpu.make_async_copy(wout_hbm, wout_v, wsem.at[5])

    x_copy(0).start()
    wq_cp.start()
    for i in range(1, NT):
        x_copy(i).start()
    wo_cp.start()
    win_cp.start()
    bsp_cp.start()
    wout_cp.start()
    wsp_cp.start()

    kv_v[...] = jnp.zeros(kv_v.shape, f32)
    zs_v[...] = jnp.zeros(zs_v.shape, f32)

    wq_cp.wait()

    def p1(i, carry):
        r = pl.multiple_of(i * TM, TM)
        x_copy(i).wait()
        x = x_v[pl.ds(r, TM), :].astype(f32)
        xn = _ln(x).astype(bf16)
        qkv = jnp.dot(xn, wqkv_v[...], preferred_element_type=f32)
        pq = _phi(qkv[:, :D])
        pk = _phi(qkv[:, D:2 * D])
        v = qkv[:, 2 * D:]
        pq_v[pl.ds(r, TM), :] = pq.astype(bf16)
        pkb = pk.astype(bf16)
        vb = v.astype(bf16)
        for g in range(4):
            kv_v[g] += lax.dot_general(
                pkb[:, g * 128:(g + 1) * 128], vb[:, g * 128:(g + 1) * 128],
                (((0,), (0,)), ((), ())), preferred_element_type=f32)
        zs_v[...] += jnp.sum(pk, axis=0, keepdims=True)
        return carry

    lax.fori_loop(0, NT, p1, 0)

    wo_cp.wait()
    row = lax.broadcasted_iota(jnp.int32, (128, 128), 0) // DH
    col = lax.broadcasted_iota(jnp.int32, (128, 128), 1) // DH
    mask = row == col
    for g in range(4):
        kvm = jnp.where(mask, kv_v[g], 0.0).astype(bf16)
        m_v[g * 128:(g + 1) * 128, :] = jnp.dot(
            kvm, wo_v[g * 128:(g + 1) * 128, :], preferred_element_type=f32).astype(bf16)
    ones_bd = jnp.where(mask, 1.0, 0.0).astype(bf16)
    zrow = zs_v[...]

    bsp_cp.wait()
    b = bsp_v[...].astype(f32)
    for j in range(16):
        bj = jnp.broadcast_to(b[j:j + 1, :], (128, 128))
        bcol_v[j * 128:(j + 1) * 128, :] = bj.T

    win_cp.wait()

    def p2(i, carry):
        r = pl.multiple_of(i * TM, TM)
        pq = pq_v[pl.ds(r, TM), :].astype(f32)
        t = (pq * zrow).astype(bf16)
        den = jnp.concatenate(
            [jnp.dot(t[:, g * 128:(g + 1) * 128], ones_bd, preferred_element_type=f32)
             for g in range(4)], axis=1) + 1e-6
        rr = (pq / den).astype(bf16)
        attn = jnp.dot(rr, m_v[...], preferred_element_type=f32)
        h = x_v[pl.ds(r, TM), :].astype(f32) + attn
        h_v[pl.ds(r, TM), :] = h
        hn = _ln(h).astype(bf16)
        zz = _gelu(jnp.dot(hn, win_v[...], preferred_element_type=f32))
        z1_v[pl.ds(r, TM), :] = zz[:, :FH].astype(bf16)
        z2_v[pl.ds(r, TM), :] = _ln(zz[:, FH:]).astype(bf16)
        return carry

    lax.fori_loop(0, NT, p2, 0)

    wout_cp.wait()
    wsp_cp.wait()

    def o_copy(i, slot):
        r = pl.multiple_of(i * TM, TM)
        return pltpu.make_async_copy(o_v.at[slot], o_hbm.at[0, pl.ds(r, TM), :], osem.at[slot])

    def p3(i, carry):
        r = pl.multiple_of(i * TM, TM)
        slot = i % 2
        g = jnp.dot(wsp_v[pl.ds(r, TM), :], z2_v[...], preferred_element_type=f32)
        bc = bcol_v[pl.ds(r, TM), :]
        g = g + jnp.concatenate([bc] * 7, axis=1)
        u = (z1_v[pl.ds(r, TM), :].astype(f32) * g).astype(bf16)
        out = jnp.dot(u, wout_v[...], preferred_element_type=f32) + h_v[pl.ds(r, TM), :]

        @pl.when(i >= 2)
        def _():
            o_copy(i - 2, slot).wait()

        o_v[slot] = out.astype(bf16)
        o_copy(i, slot).start()
        return carry

    lax.fori_loop(0, NT, p3, 0)
    o_copy(NT - 2, (NT - 2) % 2).wait()
    o_copy(NT - 1, (NT - 1) % 2).wait()


@jax.jit
def pallas_sequential_preLN__linear_attn_block__mixer_gmlp__prompt_kernel(
    A_x: jax.Array,
    A_wqkv: jax.Array,
    A_wo: jax.Array,
    B_x: jax.Array,
    B_w_in: jax.Array,
    B_w_sp: jax.Array,
    B_b_sp: jax.Array,
    B_w_out: jax.Array,
):
    any_spec = pl.BlockSpec(memory_space=pl.ANY)
    return pl.pallas_call(
        _kernel,
        out_shape=jax.ShapeDtypeStruct((1, S, D), bf16),
        in_specs=[any_spec] * 7,
        out_specs=any_spec,
        scratch_shapes=[
            pltpu.VMEM((S, D), bf16),
            pltpu.VMEM((D, 3 * D), bf16),
            pltpu.VMEM((D, D), bf16),
            pltpu.VMEM((D, F), bf16),
            pltpu.VMEM((S, S), bf16),
            pltpu.VMEM((16, 128), bf16),
            pltpu.VMEM((FH, D), bf16),
            pltpu.VMEM((S, D), bf16),
            pltpu.VMEM((S, D), f32),
            pltpu.VMEM((S, FH), bf16),
            pltpu.VMEM((S, FH), bf16),
            pltpu.VMEM((4, 128, 128), f32),
            pltpu.VMEM((1, D), f32),
            pltpu.VMEM((D, D), bf16),
            pltpu.VMEM((S, 128), f32),
            pltpu.VMEM((2, TM, D), bf16),
            pltpu.SemaphoreType.DMA((NT,)),
            pltpu.SemaphoreType.DMA((6,)),
            pltpu.SemaphoreType.DMA((2,)),
        ],
        compiler_params=pltpu.CompilerParams(vmem_limit_bytes=100 * 1024 * 1024),
    )(A_x, A_wqkv, A_wo, B_w_in, B_w_sp, B_b_sp.reshape(16, 128), B_w_out)
```

```python
import jax
import jax.numpy as jnp
from jax import lax
import jax.experimental.pallas as pl
import jax.experimental.pallas.tpu as pltpu

S, D, H, DH = 2048, 512, 32, 16
F = 1792
FH = 896
TM = 256
NT = S // TM
f32 = jnp.float32
bf16 = jnp.bfloat16


def _ln(x):
    m = jnp.mean(x, axis=-1, keepdims=True)
    xc = x - m
    v = jnp.mean(xc * xc, axis=-1, keepdims=True)
    return xc * lax.rsqrt(v + 1e-5)


def _phi(t):
    return jnp.where(t > 0, t + 1.0, jnp.exp(t)) + 1e-6


def _gelu(x):
    c = 0.7978845608028654
    a = x * (c + (c * 0.044715) * (x * x))
    return x * (0.5 + 0.5 * jnp.tanh(a))


def _recip(d):
    r = pl.reciprocal(d, approx=True)
    return r * (2.0 - d * r)


def _kernel(x_hbm, wqkv_hbm, wo_hbm, win_hbm, wsp_hbm, bsp_hbm, wout_hbm, o_hbm,
            x_v, wqkv_v, wo_v, win_v, wsp_v, bsp_v, wout_v,
            pq_v, h_v, z1_v, g_v, m_v, bcol_v, o_v, wqp_v,
            xsem, wsem, osem):
    def rows(i):
        return pl.ds(i * TM, TM)

    def x_copy(i):
        return pltpu.make_async_copy(x_hbm.at[0, rows(i), :], x_v.at[rows(i), :], xsem.at[i])

    def w3_copy(c):
        return pltpu.make_async_copy(wqkv_hbm.at[:, pl.ds(c * D, D)], wqkv_v.at[:, pl.ds(c * D, D)],
                                     wsem.at[6 + c])

    wo_cp = pltpu.make_async_copy(wo_hbm, wo_v, wsem.at[1])
    win_cp = pltpu.make_async_copy(win_hbm, win_v, wsem.at[2])
    wsp_cp = pltpu.make_async_copy(wsp_hbm, wsp_v, wsem.at[3])
    bsp_cp = pltpu.make_async_copy(bsp_hbm, bsp_v, wsem.at[4])
    wout_cp = pltpu.make_async_copy(wout_hbm, wout_v, wsem.at[5])

    x_copy(0).start()
    x_copy(1).start()
    w3_copy(1).start()
    w3_copy(2).start(priority=1)

    def ln_x(i):
        return _ln(x_v[rows(i), :].astype(f32)).astype(bf16)

    def q_proj(xn, i, c0, c1):
        q = jnp.dot(xn, wqp_v[:, c0:c1], preferred_element_type=f32)
        pq_v[rows(i), c0:c1] = _phi(q).astype(bf16)

    r_i = lax.broadcasted_iota(jnp.int32, (128, 128), 0)
    c_i = lax.broadcasted_iota(jnp.int32, (128, 128), 1)
    perm = c_i == (r_i % DH) * 8 + r_i // DH
    perm_t = r_i == (c_i % DH) * 8 + c_i // DH
    p_b = jnp.where(perm, 1.0, 0.0).astype(bf16)
    pt_b = jnp.where(perm_t, 1.0, 0.0).astype(bf16)

    st = {'kv': [None] * 4, 'zs': None}

    def k_proj(xn):
        return jnp.dot(xn, wqkv_v[:, D:2 * D], preferred_element_type=f32)

    def v_proj(xn):
        return jnp.dot(xn, wqkv_v[:, 2 * D:], preferred_element_type=f32)

    def phi_k(k):
        pk = _phi(k)
        s = jnp.sum(pk, axis=0, keepdims=True)
        st['zs'] = s if st['zs'] is None else st['zs'] + s
        return pk.astype(bf16)

    def kv_acc(pkb, v):
        vb = v.astype(bf16)
        kv = st['kv']
        for g in range(4):
            c = lax.dot_general(
                pkb[:, g * 128:(g + 1) * 128], vb[:, g * 128:(g + 1) * 128],
                (((0,), (0,)), ((), ())), preferred_element_type=f32)
            kv[g] = c if kv[g] is None else kv[g] + c

    xns = [None] * NT
    x_copy(0).wait()
    xns[0] = ln_x(0)
    x_copy(1).wait()
    w3_copy(1).wait()
    w3_copy(0).start(priority=1)
    k0 = k_proj(xns[0])
    xns[1] = ln_x(1)
    k1 = k_proj(xns[1])
    pk0 = phi_k(k0)
    w3_copy(2).wait()
    x_copy(2).start()
    x_copy(3).start()
    wsp_cp.start(priority=1)
    v0 = v_proj(xns[0])
    pk1 = phi_k(k1)
    v1 = v_proj(xns[1])
    kv_acc(pk0, v0)
    w3_copy(0).wait()
    x_copy(2).wait()
    x_copy(3).wait()
    for t in range(4, NT):
        x_copy(t).start()
    wo_cp.start()
    for g in range(4):
        wqp_v[:, g * 128:(g + 1) * 128] = jnp.dot(
            wqkv_v[:, g * 128:(g + 1) * 128], p_b, preferred_element_type=f32).astype(bf16)
    q_proj(xns[0], 0, 0, D)
    kv_acc(pk1, v1)
    xns[2] = ln_x(2)
    q_proj(xns[1], 1, 0, D)

    def perm_z(zs):
        z_hi = zs.astype(bf16)
        z_r = zs - z_hi.astype(f32)
        z_mid = z_r.astype(bf16)
        z_lo = (z_r - z_mid.astype(f32)).astype(bf16)
        sub = lax.broadcasted_iota(jnp.int32, (8, D), 0)
        z3 = jnp.where(sub == 0, z_hi.astype(f32),
                       jnp.where(sub == 1, z_mid.astype(f32),
                                 jnp.where(sub == 2, z_lo.astype(f32), 0.0))).astype(bf16)
        return jnp.concatenate(
            [jnp.sum(jnp.dot(z3[:, g * 128:(g + 1) * 128], p_b, preferred_element_type=f32),
                     axis=0, keepdims=True) for g in range(4)], axis=1)

    DEFER = (5, 6, 7)
    for i in range(2, NT):
        xn = xns[i]
        if i == 3:
            for t in range(4, NT):
                x_copy(t).wait()
            wo_cp.wait()
            bsp_cp.start()
            win_cp.start()
        k = k_proj(xn)
        v = v_proj(xn)
        pk = phi_k(k)
        if i not in DEFER:
            q_proj(xn, i, 0, D)
        elif i == NT - 1:
            q_proj(xn, i, 0, D // 2)
            zrow = perm_z(st['zs'])
        if i + 1 < NT:
            xns[i + 1] = ln_x(i + 1)
        kv_acc(pk, v)
    kv = st['kv']

    row = lax.broadcasted_iota(jnp.int32, (128, 128), 0) // DH
    col = lax.broadcasted_iota(jnp.int32, (128, 128), 1) // DH
    mask = row == col

    def den_rr(i):
        pq = pq_v[rows(i), :].astype(f32)
        t = pq * zrow
        outs = []
        for g in range(4):
            tg = t[:, g * 128:(g + 1) * 128]
            for sh in (64, 32, 16, 8):
                tg = tg + pltpu.roll(tg, sh, 1)
            outs.append(tg)
        den = jnp.concatenate(outs, axis=1) + 1e-6
        return (pq * _recip(den)).astype(bf16)

    def attn_hn(rr, i):
        attn = jnp.dot(rr, m_v[...], preferred_element_type=f32)
        h = x_v[rows(i), :].astype(f32) + attn
        h_v[rows(i), :] = h
        return _ln(h).astype(bf16)

    def w_in(hn, i):
        d2 = jnp.dot(hn, win_v[:, FH:], preferred_element_type=f32)
        zz2 = _gelu(d2)
        zz1 = _gelu(jnp.dot(hn, win_v[:, :FH], preferred_element_type=f32))
        z1_v[rows(i), :] = zz1.astype(bf16)
        return _ln(zz2).astype(bf16)

    def g_blocks(z2, j, b0, b1):
        for b in range(b0, b1):
            c = jnp.dot(wsp_v[rows(b), rows(j)], z2, preferred_element_type=f32)
            if j == 0:
                g_v[rows(b), :] = c
            else:
                g_v[rows(b), :] += c

    rrs = [None] * NT
    rrs[0] = den_rr(0)

    q_proj(xns[7], 7, D // 2, D)
    kvp = []
    for g in range(4):
        kvm = jnp.where(mask, kv[g], 0.0).astype(bf16)
        kvp.append(jnp.dot(pt_b, kvm, preferred_element_type=f32).astype(bf16))
    q_proj(xns[5], 5, 0, D // 2)
    for g in range(4):
        m_v[g * 128:(g + 1) * 128, :] = jnp.dot(
            kvp[g], wo_v[g * 128:(g + 1) * 128, :], preferred_element_type=f32).astype(bf16)
    q_proj(xns[5], 5, D // 2, D)
    hn = attn_hn(rrs[0], 0)
    q_proj(xns[6], 6, 0, D)
    wsp_cp.wait()
    bsp_cp.wait()
    win_cp.wait()
    wout_cp.start()
    rrs[1] = den_rr(1)
    z2 = w_in(hn, 0)
    z2_prev = None
    for j in range(NT - 1):
        hn = attn_hn(rrs[j + 1], j + 1)
        g_blocks(z2, j, 0, 1)
        if j + 2 < NT:
            rrs[j + 2] = den_rr(j + 2)
        if j + 1 < NT - 1:
            g_blocks(z2, j, 1, 5)
            if j == 2:
                wout_cp.wait()
                b = bsp_v[...].astype(f32)
                for jj in range(16):
                    bj = jnp.broadcast_to(b[jj:jj + 1, :], (128, 128))
                    bcol_v[jj * 128:(jj + 1) * 128, :] = bj.T
            g_blocks(z2, j, 5, NT)
            z2 = w_in(hn, j + 1)
        else:
            g_blocks(z2, j, 1, NT - 1)
            z2n = w_in(hn, j + 1)
            g_blocks(z2, j, NT - 1, NT)
            z2 = z2n

    def o_copy(r0, n, s):
        return pltpu.make_async_copy(o_v.at[pl.ds(r0, n), :], o_hbm.at[0, pl.ds(r0, n), :], osem.at[s])

    pieces = []
    for i in range(NT):
        g = g_v[rows(i), :] + jnp.dot(wsp_v[rows(i), rows(NT - 1)], z2,
                                      preferred_element_type=f32)
        bc = bcol_v[rows(i), :]
        g = g + jnp.concatenate([bc] * 7, axis=1)
        u = (z1_v[rows(i), :].astype(f32) * g).astype(bf16)
        nsplit = 2 if i == NT - 1 else 1
        n = TM // nsplit
        for p in range(nsplit):
            r0 = i * TM + p * n
            out = jnp.dot(u[p * n:(p + 1) * n], wout_v[...], preferred_element_type=f32) + h_v[pl.ds(r0, n), :]
            o_v[pl.ds(r0, n), :] = out.astype(bf16)
            pieces.append((r0, n, len(pieces)))
            o_copy(*pieces[-1]).start()
    for pc in pieces:
        o_copy(*pc).wait()


@jax.jit
def pallas_sequential_preLN__linear_attn_block__mixer_gmlp__prompt_kernel(
    A_x: jax.Array,
    A_wqkv: jax.Array,
    A_wo: jax.Array,
    B_x: jax.Array,
    B_w_in: jax.Array,
    B_w_sp: jax.Array,
    B_b_sp: jax.Array,
    B_w_out: jax.Array,
):
    any_spec = pl.BlockSpec(memory_space=pl.ANY)
    return pl.pallas_call(
        _kernel,
        out_shape=jax.ShapeDtypeStruct((1, S, D), bf16),
        in_specs=[any_spec] * 7,
        out_specs=any_spec,
        scratch_shapes=[
            pltpu.VMEM((S, D), bf16),
            pltpu.VMEM((D, 3 * D), bf16),
            pltpu.VMEM((D, D), bf16),
            pltpu.VMEM((D, F), bf16),
            pltpu.VMEM((S, S), bf16),
            pltpu.VMEM((16, 128), bf16),
            pltpu.VMEM((FH, D), bf16),
            pltpu.VMEM((S, D), bf16),
            pltpu.VMEM((S, D), f32),
            pltpu.VMEM((S, FH), bf16),
            pltpu.VMEM((S, FH), f32),
            pltpu.VMEM((D, D), bf16),
            pltpu.VMEM((S, 128), f32),
            pltpu.VMEM((S, D), bf16),
            pltpu.VMEM((D, D), bf16),
            pltpu.SemaphoreType.DMA((NT,)),
            pltpu.SemaphoreType.DMA((9,)),
            pltpu.SemaphoreType.DMA((NT + 1,)),
        ],
        compiler_params=pltpu.CompilerParams(vmem_limit_bytes=100 * 1024 * 1024),
    )(A_x, A_wqkv, A_wo, B_w_in, B_w_sp, B_b_sp.reshape(16, 128), B_w_out)
```

```python
import jax
import jax.numpy as jnp
from jax import lax
import jax.experimental.pallas as pl
import jax.experimental.pallas.tpu as pltpu

S, D, H, DH = 2048, 512, 32, 16
F = 1792
FH = 896
TM = 256
NT = S // TM
HS = S // 2
f32 = jnp.float32
bf16 = jnp.bfloat16


def _ln(x):
    m = jnp.mean(x, axis=-1, keepdims=True)
    xc = x - m
    v = jnp.mean(xc * xc, axis=-1, keepdims=True)
    return xc * lax.rsqrt(v + 1e-5)


def _phi(t):
    return jnp.where(t > 0, t + 1.0, jnp.exp(t)) + 1e-6


def _gelu(x):
    c = 0.7978845608028654
    a = x * (c + (c * 0.044715) * (x * x))
    return x * (0.5 + 0.5 * jnp.tanh(a))


def _recip(d):
    r = pl.reciprocal(d, approx=True)
    return r * (2.0 - d * r)


def _kernel(x_hbm, wqkv_hbm, wo_hbm, win_hbm, wsp_hbm, bsp_hbm, wout_hbm, o_hbm,
            x_v, wqkv_v, wo_v, win_v, wsp_v, bsp_v, wout_v,
            pq_v, h_v, z1_v, g_v, m_v, bcol_v, o_v,
            xsem, wsem, osem):
    def rows(i):
        return pl.ds(i * TM, TM)

    def x_copy(i):
        return pltpu.make_async_copy(x_hbm.at[0, rows(i), :], x_v.at[rows(i), :], xsem.at[i])

    def w3_copy(c):
        return pltpu.make_async_copy(wqkv_hbm.at[:, pl.ds(c * D, D)], wqkv_v.at[:, pl.ds(c * D, D)],
                                     wsem.at[6 + c])

    wo_cp = pltpu.make_async_copy(wo_hbm, wo_v, wsem.at[1])
    win_cp = pltpu.make_async_copy(win_hbm, win_v, wsem.at[2])
    wsp_cp = pltpu.make_async_copy(wsp_hbm.at[:, pl.ds(0, HS)], wsp_v.at[:, pl.ds(0, HS)], wsem.at[3])
    wsp2_cp = pltpu.make_async_copy(wsp_hbm.at[:, pl.ds(HS, HS)], wsp_v.at[:, pl.ds(HS, HS)], wsem.at[0])
    bsp_cp = pltpu.make_async_copy(bsp_hbm, bsp_v, wsem.at[4])
    wout_cp = pltpu.make_async_copy(wout_hbm, wout_v, wsem.at[5])

    x_copy(0).start()
    x_copy(1).start()
    w3_copy(1).start()

    def ln_x(i):
        return _ln(x_v[rows(i), :].astype(f32)).astype(bf16)

    def q_proj(xn, i, c0, c1):
        q = jnp.dot(xn, wqkv_v[:, c0:c1], preferred_element_type=f32)
        pq_v[rows(i), c0:c1] = _phi(q).astype(bf16)

    st = {'kv': [None] * 4, 'zs': None}

    def k_proj(xn):
        return jnp.dot(xn, wqkv_v[:, D:2 * D], preferred_element_type=f32)

    def v_proj(xn):
        return jnp.dot(xn, wqkv_v[:, 2 * D:], preferred_element_type=f32)

    def phi_k(k):
        pk = _phi(k)
        s = jnp.sum(pk, axis=0, keepdims=True)
        st['zs'] = s if st['zs'] is None else st['zs'] + s
        return pk.astype(bf16)

    def kv_acc(pkb, v):
        vb = v.astype(bf16)
        kv = st['kv']
        for g in range(4):
            c = lax.dot_general(
                pkb[:, g * 128:(g + 1) * 128], vb[:, g * 128:(g + 1) * 128],
                (((0,), (0,)), ((), ())), preferred_element_type=f32)
            kv[g] = c if kv[g] is None else kv[g] + c

    xns = [None] * NT
    x_copy(0).wait()
    xns[0] = ln_x(0)
    x_copy(1).wait()
    w3_copy(1).wait()
    w3_copy(2).start()
    w3_copy(0).start(priority=1)
    k0 = k_proj(xns[0])
    xns[1] = ln_x(1)
    k1 = k_proj(xns[1])
    pk0 = phi_k(k0)
    w3_copy(2).wait()
    x_copy(2).start()
    x_copy(3).start()
    v0 = v_proj(xns[0])
    pk1 = phi_k(k1)
    v1 = v_proj(xns[1])
    kv_acc(pk0, v0)
    w3_copy(0).wait()
    x_copy(2).wait()
    x_copy(3).wait()
    for t in range(4, NT):
        x_copy(t).start()
    wo_cp.start()
    wsp_cp.start(priority=1)
    q_proj(xns[0], 0, 0, D)
    kv_acc(pk1, v1)
    xns[2] = ln_x(2)
    q_proj(xns[1], 1, 0, D)

    DEFER = (5, 6, 7)
    for i in range(2, NT):
        xn = xns[i]
        if i == 3:
            for t in range(4, NT):
                x_copy(t).wait()
            wo_cp.wait()
            bsp_cp.start()
            win_cp.start()
        k = k_proj(xn)
        v = v_proj(xn)
        pk = phi_k(k)
        if i not in DEFER:
            q_proj(xn, i, 0, D)
        elif i == NT - 1:
            q_proj(xn, i, 0, D // 2)
        if i + 1 < NT:
            xns[i + 1] = ln_x(i + 1)
        kv_acc(pk, v)
    kv = st['kv']
    zrow = st['zs']

    row = lax.broadcasted_iota(jnp.int32, (128, 128), 0) // DH
    col = lax.broadcasted_iota(jnp.int32, (128, 128), 1) // DH
    mask = row == col
    lane0 = lax.broadcasted_iota(jnp.int32, (TM, 128), 1) % DH == 0

    def den_rr(i):
        pq = pq_v[rows(i), :].astype(f32)
        t = pq * zrow
        outs = []
        for g in range(4):
            tg = t[:, g * 128:(g + 1) * 128]
            for sh in (1, 2, 4, 8):
                tg = tg + pltpu.roll(tg, 128 - sh, 1)
            tg = jnp.where(lane0, tg, 0.0)
            for sh in (1, 2, 4, 8):
                tg = tg + pltpu.roll(tg, sh, 1)
            outs.append(tg)
        den = jnp.concatenate(outs, axis=1) + 1e-6
        return (pq * _recip(den)).astype(bf16)

    def attn_hn(rr, i):
        attn = jnp.dot(rr, m_v[...], preferred_element_type=f32)
        if i == 4:
            wsp2_cp.wait()
            wout_cp.wait()
        h = x_v[rows(i), :].astype(f32) + attn
        h_v[rows(i), :] = h
        return _ln(h).astype(bf16)

    def w_in(hn, i):
        d2 = jnp.dot(hn, win_v[:, FH:], preferred_element_type=f32)
        zz2 = _gelu(d2)
        zz1 = jnp.dot(hn, win_v[:, :FH], preferred_element_type=f32)
        z1_v[rows(i), :] = zz1.astype(bf16)
        return _ln(zz2).astype(bf16)

    def g_blocks(z2, j, b0, b1):
        for b in range(b0, b1):
            c = jnp.dot(wsp_v[rows(b), rows(j)], z2, preferred_element_type=f32)
            if j == 0:
                g_v[rows(b), :] = c
            else:
                g_v[rows(b), :] += c

    rrs = [None] * NT
    rrs[0] = den_rr(0)

    q_proj(xns[7], 7, D // 2, D)
    kvm = [jnp.where(mask, kv[g], 0.0).astype(bf16) for g in range(4)]
    q_proj(xns[5], 5, 0, D // 2)
    for g in range(4):
        m_v[g * 128:(g + 1) * 128, :] = jnp.dot(
            kvm[g], wo_v[g * 128:(g + 1) * 128, :], preferred_element_type=f32).astype(bf16)
    q_proj(xns[5], 5, D // 2, D)
    hn = attn_hn(rrs[0], 0)
    q_proj(xns[6], 6, 0, D)
    wsp_cp.wait()
    bsp_cp.wait()
    win_cp.wait()
    wsp2_cp.start()
    wout_cp.start()
    rrs[1] = den_rr(1)
    z2 = w_in(hn, 0)
    for j in range(NT - 1):
        hn = attn_hn(rrs[j + 1], j + 1)
        g_blocks(z2, j, 0, 1)
        if j + 2 < NT:
            rrs[j + 2] = den_rr(j + 2)
        if j + 1 < NT - 1:
            g_blocks(z2, j, 1, 5)
            if j == 3:
                b = bsp_v[...].astype(f32)
                for jj in range(16):
                    bj = jnp.broadcast_to(b[jj:jj + 1, :], (128, 128))
                    bcol_v[jj * 128:(jj + 1) * 128, :] = bj.T
            g_blocks(z2, j, 5, NT)
            z2 = w_in(hn, j + 1)
        else:
            g_blocks(z2, j, 1, NT - 1)
            z2n = w_in(hn, j + 1)
            g_blocks(z2, j, NT - 1, NT)
            z2 = z2n

    def o_copy(r0, n, s):
        return pltpu.make_async_copy(o_v.at[pl.ds(r0, n), :], o_hbm.at[0, pl.ds(r0, n), :], osem.at[s])

    pieces = []
    for i in range(NT):
        g = g_v[rows(i), :] + jnp.dot(wsp_v[rows(i), rows(NT - 1)], z2,
                                      preferred_element_type=f32)
        bc = bcol_v[rows(i), :]
        g = g + jnp.concatenate([bc] * 7, axis=1)
        u = (_gelu(z1_v[rows(i), :].astype(f32)) * g).astype(bf16)
        nsplit = 2 if i == NT - 1 else 1
        n = TM // nsplit
        for p in range(nsplit):
            r0 = i * TM + p * n
            out = jnp.dot(u[p * n:(p + 1) * n], wout_v[...],
                          preferred_element_type=f32) + h_v[pl.ds(r0, n), :]
            o_v[pl.ds(r0, n), :] = out.astype(bf16)
            pieces.append((r0, n, len(pieces)))
            o_copy(*pieces[-1]).start()
    for pc in pieces:
        o_copy(*pc).wait()


@jax.jit
def pallas_sequential_preLN__linear_attn_block__mixer_gmlp__prompt_kernel(
    A_x: jax.Array,
    A_wqkv: jax.Array,
    A_wo: jax.Array,
    B_x: jax.Array,
    B_w_in: jax.Array,
    B_w_sp: jax.Array,
    B_b_sp: jax.Array,
    B_w_out: jax.Array,
):
    any_spec = pl.BlockSpec(memory_space=pl.ANY)
    return pl.pallas_call(
        _kernel,
        out_shape=jax.ShapeDtypeStruct((1, S, D), bf16),
        in_specs=[any_spec] * 7,
        out_specs=any_spec,
        scratch_shapes=[
            pltpu.VMEM((S, D), bf16),
            pltpu.VMEM((D, 3 * D), bf16),
            pltpu.VMEM((D, D), bf16),
            pltpu.VMEM((D, F), bf16),
            pltpu.VMEM((S, S), bf16),
            pltpu.VMEM((16, 128), bf16),
            pltpu.VMEM((FH, D), bf16),
            pltpu.VMEM((S, D), bf16),
            pltpu.VMEM((S, D), f32),
            pltpu.VMEM((S, FH), bf16),
            pltpu.VMEM((S, FH), f32),
            pltpu.VMEM((D, D), bf16),
            pltpu.VMEM((S, 128), f32),
            pltpu.VMEM((S, D), bf16),
            pltpu.SemaphoreType.DMA((NT,)),
            pltpu.SemaphoreType.DMA((9,)),
            pltpu.SemaphoreType.DMA((NT + 1,)),
        ],
        compiler_params=pltpu.CompilerParams(vmem_limit_bytes=100 * 1024 * 1024),
    )(A_x, A_wqkv, A_wo, B_w_in, B_w_sp, B_b_sp.reshape(16, 128), B_w_out)
```

```python
import jax
import jax.numpy as jnp
from jax import lax
import jax.experimental.pallas as pl
import jax.experimental.pallas.tpu as pltpu

S, D, H, DH = 2048, 512, 32, 16
F = 1792
FH = 896
TM = 256
NT = S // TM
HS = S // 2
NSPLIT = 4
f32 = jnp.float32
bf16 = jnp.bfloat16


def _ln(x):
    m = jnp.mean(x, axis=-1, keepdims=True)
    xc = x - m
    v = jnp.mean(xc * xc, axis=-1, keepdims=True)
    return xc * lax.rsqrt(v + 1e-5)


def _phi(t):
    return jnp.where(t > 0, t + 1.0, jnp.exp(t)) + 1e-6


def _gelu(x):
    c = 0.7978845608028654
    a = x * (c + (c * 0.044715) * (x * x))
    return x * (0.5 + 0.5 * jnp.tanh(a))


def _recip(d):
    r = pl.reciprocal(d, approx=True)
    return r * (2.0 - d * r)


def _kernel(x_hbm, wqkv_hbm, wo_hbm, win_hbm, wsp_hbm, bsp_hbm, wout_hbm, o_hbm,
            x_v, wqkv_v, wo_v, win_v, wsp_v, bsp_v, wout_v,
            pq_v, h_v, z1_v, g_v, m_v, bcol_v, o_v,
            xsem, wsem, osem):
    def rows(i):
        return pl.ds(i * TM, TM)

    def x_copy(i):
        return pltpu.make_async_copy(x_hbm.at[0, rows(i), :], x_v.at[rows(i), :], xsem.at[i])

    def w3_copy(c):
        return pltpu.make_async_copy(wqkv_hbm.at[:, pl.ds(c * D, D)], wqkv_v.at[:, pl.ds(c * D, D)],
                                     wsem.at[6 + c])

    wo_cp = pltpu.make_async_copy(wo_hbm, wo_v, wsem.at[1])
    win_cp = pltpu.make_async_copy(win_hbm, win_v, wsem.at[2])
    wsp_cp = pltpu.make_async_copy(wsp_hbm.at[:, pl.ds(0, HS)], wsp_v.at[:, pl.ds(0, HS)], wsem.at[3])
    wsp2_cp = pltpu.make_async_copy(wsp_hbm.at[:, pl.ds(HS, HS)], wsp_v.at[:, pl.ds(HS, HS)], wsem.at[0])
    bsp_cp = pltpu.make_async_copy(bsp_hbm, bsp_v, wsem.at[4])
    wout_cp = pltpu.make_async_copy(wout_hbm, wout_v, wsem.at[5])

    x_copy(0).start()
    x_copy(1).start()
    w3_copy(1).start()

    def ln_x(i):
        return _ln(x_v[rows(i), :].astype(f32)).astype(bf16)

    def q_proj(xn, i, c0, c1):
        q = jnp.dot(xn, wqkv_v[:, c0:c1], preferred_element_type=f32)
        pq_v[rows(i), c0:c1] = _phi(q).astype(bf16)

    st = {'kv': [None] * 4, 'zs': None}

    def k_proj(xn):
        return jnp.dot(xn, wqkv_v[:, D:2 * D], preferred_element_type=f32)

    def v_proj(xn):
        return jnp.dot(xn, wqkv_v[:, 2 * D:], preferred_element_type=f32)

    def phi_k(k):
        pk = _phi(k)
        s = jnp.sum(pk, axis=0, keepdims=True)
        st['zs'] = s if st['zs'] is None else st['zs'] + s
        return pk.astype(bf16)

    def kv_acc(pkb, v):
        vb = v.astype(bf16)
        kv = st['kv']
        for g in range(4):
            c = lax.dot_general(
                pkb[:, g * 128:(g + 1) * 128], vb[:, g * 128:(g + 1) * 128],
                (((0,), (0,)), ((), ())), preferred_element_type=f32)
            kv[g] = c if kv[g] is None else kv[g] + c

    xns = [None] * NT
    x_copy(0).wait()
    xns[0] = ln_x(0)
    x_copy(1).wait()
    w3_copy(1).wait()
    w3_copy(2).start()
    w3_copy(0).start(priority=1)
    k0 = k_proj(xns[0])
    xns[1] = ln_x(1)
    k1 = k_proj(xns[1])
    pk0 = phi_k(k0)
    w3_copy(2).wait()
    x_copy(2).start()
    x_copy(3).start()
    v0 = v_proj(xns[0])
    pk1 = phi_k(k1)
    v1 = v_proj(xns[1])
    kv_acc(pk0, v0)
    w3_copy(0).wait()
    x_copy(2).wait()
    x_copy(3).wait()
    for t in range(4, NT):
        x_copy(t).start()
    wo_cp.start()
    wsp_cp.start(priority=1)
    q_proj(xns[0], 0, 0, D)
    kv_acc(pk1, v1)
    xns[2] = ln_x(2)
    q_proj(xns[1], 1, 0, D)

    DEFER = (5, 6, 7)
    for i in range(2, NT):
        xn = xns[i]
        if i == 3:
            for t in range(4, NT):
                x_copy(t).wait()
            wo_cp.wait()
            bsp_cp.start()
            win_cp.start()
        k = k_proj(xn)
        v = v_proj(xn)
        pk = phi_k(k)
        if i not in DEFER:
            q_proj(xn, i, 0, D)
        elif i == NT - 1:
            q_proj(xn, i, 0, D // 2)
        if i + 1 < NT:
            xns[i + 1] = ln_x(i + 1)
        kv_acc(pk, v)
    kv = st['kv']
    zrow = st['zs']

    row = lax.broadcasted_iota(jnp.int32, (128, 128), 0) // DH
    col = lax.broadcasted_iota(jnp.int32, (128, 128), 1) // DH
    mask = row == col
    lane0 = lax.broadcasted_iota(jnp.int32, (TM, 128), 1) % DH == 0

    def den_rr(i):
        pq = pq_v[rows(i), :].astype(f32)
        t = pq * zrow
        outs = []
        for g in range(4):
            tg = t[:, g * 128:(g + 1) * 128]
            for sh in (1, 2, 4, 8):
                tg = tg + pltpu.roll(tg, 128 - sh, 1)
            tg = jnp.where(lane0, tg, 0.0)
            for sh in (1, 2, 4, 8):
                tg = tg + pltpu.roll(tg, sh, 1)
            outs.append(tg)
        den = jnp.concatenate(outs, axis=1) + 1e-6
        return (pq * _recip(den)).astype(bf16)

    def attn_hn(rr, i):
        attn = jnp.dot(rr, m_v[...], preferred_element_type=f32)
        if i == 4:
            wsp2_cp.wait()
            wout_cp.wait()
        h = x_v[rows(i), :].astype(f32) + attn
        h_v[rows(i), :] = h
        return _ln(h).astype(bf16)

    def w_in(hn, i):
        d2 = jnp.dot(hn, win_v[:, FH:], preferred_element_type=f32)
        zz2 = _gelu(d2)
        zz1 = jnp.dot(hn, win_v[:, :FH], preferred_element_type=f32)
        z1_v[rows(i), :] = zz1.astype(bf16)
        return _ln(zz2).astype(bf16)

    def g_blocks(z2, j, b0, b1):
        for b in range(b0, b1):
            c = jnp.dot(wsp_v[rows(b), rows(j)], z2, preferred_element_type=f32)
            if j == 0:
                g_v[rows(b), :] = c
            else:
                g_v[rows(b), :] += c

    rrs = [None] * NT
    rrs[0] = den_rr(0)

    q_proj(xns[7], 7, D // 2, D)
    kvm = [jnp.where(mask, kv[g], 0.0).astype(bf16) for g in range(4)]
    q_proj(xns[5], 5, 0, D // 2)
    for g in range(4):
        m_v[g * 128:(g + 1) * 128, :] = jnp.dot(
            kvm[g], wo_v[g * 128:(g + 1) * 128, :], preferred_element_type=f32).astype(bf16)
    q_proj(xns[5], 5, D // 2, D)
    hn = attn_hn(rrs[0], 0)
    q_proj(xns[6], 6, 0, D)
    wsp_cp.wait()
    bsp_cp.wait()
    win_cp.wait()
    wsp2_cp.start()
    wout_cp.start()
    rrs[1] = den_rr(1)
    z2 = w_in(hn, 0)
    for j in range(NT - 1):
        hn = attn_hn(rrs[j + 1], j + 1)
        g_blocks(z2, j, 0, 1)
        if j + 2 < NT:
            rrs[j + 2] = den_rr(j + 2)
        if j + 1 < NT - 1:
            g_blocks(z2, j, 1, 5)
            if j == 3:
                b = bsp_v[...].astype(f32)
                for jj in range(16):
                    bj = jnp.broadcast_to(b[jj:jj + 1, :], (128, 128))
                    bcol_v[jj * 128:(jj + 1) * 128, :] = bj.T
            g_blocks(z2, j, 5, NT)
            z2 = w_in(hn, j + 1)
        else:
            g_blocks(z2, j, 1, NT - 1)
            z2n = w_in(hn, j + 1)
            g_blocks(z2, j, NT - 1, NT)
            z2 = z2n

    def o_copy(i, c0, n, s):
        return pltpu.make_async_copy(o_v.at[rows(i), pl.ds(c0, n)], o_hbm.at[0, rows(i), pl.ds(c0, n)],
                                     osem.at[s])

    pieces = []
    for i in range(NT):
        g = g_v[rows(i), :] + jnp.dot(wsp_v[rows(i), rows(NT - 1)], z2,
                                      preferred_element_type=f32)
        bc = bcol_v[rows(i), :]
        g = g + jnp.concatenate([bc] * 7, axis=1)
        u = (_gelu(z1_v[rows(i), :].astype(f32)) * g).astype(bf16)
        nsplit = NSPLIT if i == NT - 1 else 1
        n = D // nsplit
        for p in range(nsplit):
            c0 = p * n
            out = jnp.dot(u, wout_v[:, c0:c0 + n],
                          preferred_element_type=f32) + h_v[rows(i), c0:c0 + n]
            o_v[rows(i), c0:c0 + n] = out.astype(bf16)
            pieces.append((i, c0, n, len(pieces)))
            o_copy(*pieces[-1]).start()
    for pc in pieces:
        o_copy(*pc).wait()


@jax.jit
def pallas_sequential_preLN__linear_attn_block__mixer_gmlp__prompt_kernel(
    A_x: jax.Array,
    A_wqkv: jax.Array,
    A_wo: jax.Array,
    B_x: jax.Array,
    B_w_in: jax.Array,
    B_w_sp: jax.Array,
    B_b_sp: jax.Array,
    B_w_out: jax.Array,
):
    any_spec = pl.BlockSpec(memory_space=pl.ANY)
    return pl.pallas_call(
        _kernel,
        out_shape=jax.ShapeDtypeStruct((1, S, D), bf16),
        in_specs=[any_spec] * 7,
        out_specs=any_spec,
        scratch_shapes=[
            pltpu.VMEM((S, D), bf16),
            pltpu.VMEM((D, 3 * D), bf16),
            pltpu.VMEM((D, D), bf16),
            pltpu.VMEM((D, F), bf16),
            pltpu.VMEM((S, S), bf16),
            pltpu.VMEM((16, 128), bf16),
            pltpu.VMEM((FH, D), bf16),
            pltpu.VMEM((S, D), bf16),
            pltpu.VMEM((S, D), f32),
            pltpu.VMEM((S, FH), bf16),
            pltpu.VMEM((S, FH), f32),
            pltpu.VMEM((D, D), bf16),
            pltpu.VMEM((S, 128), f32),
            pltpu.VMEM((S, D), bf16),
            pltpu.SemaphoreType.DMA((NT,)),
            pltpu.SemaphoreType.DMA((9,)),
            pltpu.SemaphoreType.DMA((NT + 3,)),
        ],
        compiler_params=pltpu.CompilerParams(vmem_limit_bytes=100 * 1024 * 1024),
    )(A_x, A_wqkv, A_wo, B_w_in, B_w_sp, B_b_sp.reshape(16, 128), B_w_out)
```

```python
import jax
import jax.numpy as jnp
from jax import lax
import jax.experimental.pallas as pl
import jax.experimental.pallas.tpu as pltpu

S, D, H, DH = 2048, 512, 32, 16
F = 1792
FH = 896
TM = 256
NT = S // TM
HS = S // 2
NSPLIT = 4
f32 = jnp.float32
bf16 = jnp.bfloat16


def _ln(x):
    m = jnp.mean(x, axis=-1, keepdims=True)
    xc = x - m
    v = jnp.mean(xc * xc, axis=-1, keepdims=True)
    return xc * lax.rsqrt(v + 1e-5)


def _phi(t):
    return jnp.where(t > 0, t + 1.0, jnp.exp(t)) + 1e-6


def _gelu(x):
    c = 0.7978845608028654
    a = x * (c + (c * 0.044715) * (x * x))
    return x * (0.5 + 0.5 * jnp.tanh(a))


def _recip(d):
    r = pl.reciprocal(d, approx=True)
    return r * (2.0 - d * r)


def _kernel(x_hbm, wqkv_hbm, wo_hbm, win_hbm, wsp_hbm, bsp_hbm, wout_hbm, o_hbm,
            x_v, wqkv_v, wo_v, win_v, wsp_v, bsp_v, wout_v,
            pq_v, h_v, z1_v, g_v, m_v, bcol_v, o_v,
            xsem, wsem, osem):
    def rows(i):
        return pl.ds(i * TM, TM)

    def x_copy(i):
        return pltpu.make_async_copy(x_hbm.at[0, rows(i), :], x_v.at[rows(i), :], xsem.at[i])

    def w3_copy(c):
        return pltpu.make_async_copy(wqkv_hbm.at[:, pl.ds(c * D, D)], wqkv_v.at[:, pl.ds(c * D, D)],
                                     wsem.at[6 + c])

    wo_cp = pltpu.make_async_copy(wo_hbm, wo_v, wsem.at[1])
    win_cp = pltpu.make_async_copy(win_hbm, win_v, wsem.at[2])
    wsp_cp = pltpu.make_async_copy(wsp_hbm.at[:, pl.ds(0, HS)], wsp_v.at[:, pl.ds(0, HS)], wsem.at[3])
    wsp2_cp = pltpu.make_async_copy(wsp_hbm.at[:, pl.ds(HS, HS)], wsp_v.at[:, pl.ds(HS, HS)], wsem.at[0])
    bsp_cp = pltpu.make_async_copy(bsp_hbm, bsp_v, wsem.at[4])
    wout_cp = pltpu.make_async_copy(wout_hbm, wout_v, wsem.at[5])

    x_copy(0).start()
    w3_copy(1).start()
    x_copy(1).start(priority=1)

    def ln_x(i):
        return _ln(x_v[rows(i), :].astype(f32)).astype(bf16)

    def q_proj(xn, i, c0, c1):
        q = jnp.dot(xn, wqkv_v[:, c0:c1], preferred_element_type=f32)
        pq_v[rows(i), c0:c1] = _phi(q).astype(bf16)

    st = {'kv': [None] * 4, 'zs': None}

    def k_proj(xn):
        return jnp.dot(xn, wqkv_v[:, D:2 * D], preferred_element_type=f32)

    def v_proj(xn):
        return jnp.dot(xn, wqkv_v[:, 2 * D:], preferred_element_type=f32)

    def phi_k(k):
        pk = _phi(k)
        s = jnp.sum(pk, axis=0, keepdims=True)
        st['zs'] = s if st['zs'] is None else st['zs'] + s
        return pk.astype(bf16)

    def kv_acc(pkb, v):
        vb = v.astype(bf16)
        kv = st['kv']
        for g in range(4):
            c = lax.dot_general(
                pkb[:, g * 128:(g + 1) * 128], vb[:, g * 128:(g + 1) * 128],
                (((0,), (0,)), ((), ())), preferred_element_type=f32)
            kv[g] = c if kv[g] is None else kv[g] + c

    xns = [None] * NT
    x_copy(0).wait()
    xns[0] = ln_x(0)
    w3_copy(1).wait()
    w3_copy(2).start()
    k0a = jnp.dot(xns[0], wqkv_v[:, D:D + 256], preferred_element_type=f32)
    x_copy(1).wait()
    w3_copy(0).start(priority=1)
    k0b = jnp.dot(xns[0], wqkv_v[:, D + 256:2 * D], preferred_element_type=f32)
    k0 = jnp.concatenate([k0a, k0b], axis=1)
    xns[1] = ln_x(1)
    k1 = k_proj(xns[1])
    pk0 = phi_k(k0)
    w3_copy(2).wait()
    x_copy(2).start()
    x_copy(3).start()
    v0 = v_proj(xns[0])
    pk1 = phi_k(k1)
    v1 = v_proj(xns[1])
    kv_acc(pk0, v0)
    w3_copy(0).wait()
    x_copy(2).wait()
    x_copy(3).wait()
    for t in range(4, NT):
        x_copy(t).start()
    wo_cp.start()
    wsp_cp.start(priority=1)
    q_proj(xns[0], 0, 0, D)
    kv_acc(pk1, v1)
    xns[2] = ln_x(2)
    q_proj(xns[1], 1, 0, D)

    DEFER = (5, 6, 7)
    for i in range(2, NT):
        xn = xns[i]
        if i == 3:
            for t in range(4, NT):
                x_copy(t).wait()
            wo_cp.wait()
            bsp_cp.start()
            win_cp.start()
        k = k_proj(xn)
        v = v_proj(xn)
        pk = phi_k(k)
        if i not in DEFER:
            q_proj(xn, i, 0, D)
        elif i == NT - 1:
            q_proj(xn, i, 0, D // 2)
        if i + 1 < NT:
            xns[i + 1] = ln_x(i + 1)
        kv_acc(pk, v)
    kv = st['kv']
    zrow = st['zs']

    row = lax.broadcasted_iota(jnp.int32, (128, 128), 0) // DH
    col = lax.broadcasted_iota(jnp.int32, (128, 128), 1) // DH
    mask = row == col
    lane0 = lax.broadcasted_iota(jnp.int32, (TM, 128), 1) % DH == 0

    def den_rr(i):
        pq = pq_v[rows(i), :].astype(f32)
        t = pq * zrow
        outs = []
        for g in range(4):
            tg = t[:, g * 128:(g + 1) * 128]
            for sh in (1, 2, 4, 8):
                tg = tg + pltpu.roll(tg, 128 - sh, 1)
            tg = jnp.where(lane0, tg, 0.0)
            for sh in (1, 2, 4, 8):
                tg = tg + pltpu.roll(tg, sh, 1)
            outs.append(tg)
        den = jnp.concatenate(outs, axis=1) + 1e-6
        return (pq * _recip(den)).astype(bf16)

    def attn_hn(rr, i):
        attn = jnp.dot(rr, m_v[...], preferred_element_type=f32)
        if i == 4:
            wsp2_cp.wait()
            wout_cp.wait()
        h = x_v[rows(i), :].astype(f32) + attn
        h_v[rows(i), :] = h
        return _ln(h).astype(bf16)

    def w_in(hn, i):
        d2 = jnp.dot(hn, win_v[:, FH:], preferred_element_type=f32)
        zz2 = _gelu(d2)
        zz1 = jnp.dot(hn, win_v[:, :FH], preferred_element_type=f32)
        z1_v[rows(i), :] = zz1.astype(bf16)
        return _ln(zz2).astype(bf16)

    def g_blocks(z2, j, b0, b1):
        for b in range(b0, b1):
            c = jnp.dot(wsp_v[rows(b), rows(j)], z2, preferred_element_type=f32)
            if j == 0:
                g_v[rows(b), :] = c
            else:
                g_v[rows(b), :] += c

    rrs = [None] * NT
    rrs[0] = den_rr(0)

    q_proj(xns[7], 7, D // 2, D)
    kvm = [jnp.where(mask, kv[g], 0.0).astype(bf16) for g in range(4)]
    q_proj(xns[5], 5, 0, D // 2)
    for g in range(4):
        m_v[g * 128:(g + 1) * 128, :] = jnp.dot(
            kvm[g], wo_v[g * 128:(g + 1) * 128, :], preferred_element_type=f32).astype(bf16)
    q_proj(xns[5], 5, D // 2, D)
    hn = attn_hn(rrs[0], 0)
    q_proj(xns[6], 6, 0, D)
    wsp_cp.wait()
    bsp_cp.wait()
    win_cp.wait()
    wsp2_cp.start()
    wout_cp.start()
    rrs[1] = den_rr(1)
    z2 = w_in(hn, 0)
    for j in range(NT - 1):
        hn = attn_hn(rrs[j + 1], j + 1)
        g_blocks(z2, j, 0, 1)
        if j + 2 < NT:
            rrs[j + 2] = den_rr(j + 2)
        if j + 1 < NT - 1:
            g_blocks(z2, j, 1, 5)
            if j == 3:
                b = bsp_v[...].astype(f32)
                for jj in range(16):
                    bj = jnp.broadcast_to(b[jj:jj + 1, :], (128, 128))
                    bcol_v[jj * 128:(jj + 1) * 128, :] = bj.T
            g_blocks(z2, j, 5, NT)
            z2 = w_in(hn, j + 1)
        else:
            g_blocks(z2, j, 1, NT - 1)
            z2n = w_in(hn, j + 1)
            g_blocks(z2, j, NT - 1, NT)
            z2 = z2n

    def o_copy(i, c0, n, s):
        return pltpu.make_async_copy(o_v.at[rows(i), pl.ds(c0, n)], o_hbm.at[0, rows(i), pl.ds(c0, n)],
                                     osem.at[s])

    pieces = []
    for i in range(NT):
        g = g_v[rows(i), :] + jnp.dot(wsp_v[rows(i), rows(NT - 1)], z2,
                                      preferred_element_type=f32)
        bc = bcol_v[rows(i), :]
        g = g + jnp.concatenate([bc] * 7, axis=1)
        u = (_gelu(z1_v[rows(i), :].astype(f32)) * g).astype(bf16)
        nsplit = NSPLIT if i == NT - 1 else 1
        n = D // nsplit
        for p in range(nsplit):
            c0 = p * n
            out = jnp.dot(u, wout_v[:, c0:c0 + n],
                          preferred_element_type=f32) + h_v[rows(i), c0:c0 + n]
            o_v[rows(i), c0:c0 + n] = out.astype(bf16)
            pieces.append((i, c0, n, len(pieces)))
            o_copy(*pieces[-1]).start()
    for pc in pieces:
        o_copy(*pc).wait()


@jax.jit
def pallas_sequential_preLN__linear_attn_block__mixer_gmlp__prompt_kernel(
    A_x: jax.Array,
    A_wqkv: jax.Array,
    A_wo: jax.Array,
    B_x: jax.Array,
    B_w_in: jax.Array,
    B_w_sp: jax.Array,
    B_b_sp: jax.Array,
    B_w_out: jax.Array,
):
    any_spec = pl.BlockSpec(memory_space=pl.ANY)
    return pl.pallas_call(
        _kernel,
        out_shape=jax.ShapeDtypeStruct((1, S, D), bf16),
        in_specs=[any_spec] * 7,
        out_specs=any_spec,
        scratch_shapes=[
            pltpu.VMEM((S, D), bf16),
            pltpu.VMEM((D, 3 * D), bf16),
            pltpu.VMEM((D, D), bf16),
            pltpu.VMEM((D, F), bf16),
            pltpu.VMEM((S, S), bf16),
            pltpu.VMEM((16, 128), bf16),
            pltpu.VMEM((FH, D), bf16),
            pltpu.VMEM((S, D), bf16),
            pltpu.VMEM((S, D), f32),
            pltpu.VMEM((S, FH), bf16),
            pltpu.VMEM((S, FH), f32),
            pltpu.VMEM((D, D), bf16),
            pltpu.VMEM((S, 128), f32),
            pltpu.VMEM((S, D), bf16),
            pltpu.SemaphoreType.DMA((NT,)),
            pltpu.SemaphoreType.DMA((9,)),
            pltpu.SemaphoreType.DMA((NT + 3,)),
        ],
        compiler_params=pltpu.CompilerParams(vmem_limit_bytes=100 * 1024 * 1024),
    )(A_x, A_wqkv, A_wo, B_w_in, B_w_sp, B_b_sp.reshape(16, 128), B_w_out)
```
